```python
import os as _os
_os.environ.setdefault("JAX_PLATFORMS", "cpu")
import jax
import jax.numpy as jnp

def _softmax(x, axis=-1):
    return jax.nn.softmax(x, axis=axis)
def _gelu(x):
    return jax.nn.gelu(x, approximate=True)
def _silu(x):
    return jax.nn.silu(x)
def _sigmoid(x):
    return jax.nn.sigmoid(x)
def _layernorm(x, axis=-1, eps=1e-5):
    m = jnp.mean(x, axis=axis, keepdims=True)
    v = jnp.var(x, axis=axis, keepdims=True)
    return (x - m) / jnp.sqrt(v + eps)
def _scatter_add(tgt, idx, src, axis=0):
    return tgt.at[idx].add(src)
def _segment_sum(src, seg, n):
    return jax.ops.segment_sum(src, seg, n)
class _Rng:
    def __init__(self, key):
        self._k = key
    def _next(self):
        self._k, sub = jax.random.split(self._k)
        return sub
    def normal(self, shape):
        return jax.random.normal(self._next(), shape, dtype=jnp.bfloat16)
    def randint(self, lo, hi, shape):
        return jax.random.randint(self._next(), shape, lo, hi, dtype=jnp.int32)
    def uniform(self, shape, lo=0.0, hi=1.0):
        return jax.random.uniform(self._next(), shape, jnp.bfloat16, lo, hi)
    def permutation(self, n):
        return jax.random.permutation(self._next(), n)


kernel_name = 'gated_mix__sliding_block_cached__dense_activation_silu__decode'

def setup_inputs():
    _rng = _Rng(jax.random.key(int.from_bytes(__import__("os").urandom(4), "little")))
    _w = (lambda a: (lambda t: t.astype(jnp.bfloat16) if jnp.issubdtype(t.dtype, jnp.floating) else t)(jnp.asarray(a)))
    def _A_setup():
        B, Sq, D = 2, 1, 1024
        Hq, Hkv, Sk, Dh = 32, 4, 32768, 128
        assert Hq % Hkv == 0, (Hq, Hkv)
        return {
            "x": _w((lambda *s: _rng.normal(s) * 0.05)(B, Sq, D)),
            "k_cache": _w((lambda *s: _rng.normal(s) * 3.2)(B, Hkv, Sk, Dh)),
            "v_cache": _w((lambda *s: _rng.normal(s) * 0.05)(B, Hkv, Sk, Dh)),
            "wq": _w((lambda *s: _rng.normal(s) * 3.2)(D, Hq * Dh) * (D ** -0.5)),
            "wo": _w((lambda *s: _rng.normal(s) * 0.05)(Hq * Dh, D) * ((Hq * Dh) ** -0.5)),
        }
    _A_in = _A_setup()

    def _B_setup():
        B, S, D, F = 2, 1, 1024, 3584
        return {
            "x": _w((lambda *s: _rng.normal(s) * 0.05)(B, S, D)),
            "w1": _w((lambda *s: _rng.normal(s) * 0.05)(D, F) * (D ** -0.5)),
            "w2": _w((lambda *s: _rng.normal(s) * 0.05)(F, D) * (F ** -0.5)),
        }
    _B_in = _B_setup()

    return {
        "A_x": _A_in["x"],
        "A_k_cache": _A_in["k_cache"],
        "A_v_cache": _A_in["v_cache"],
        "A_wq": _A_in["wq"],
        "A_wo": _A_in["wo"],
        "B_x": _B_in["x"],
        "B_w1": _B_in["w1"],
        "B_w2": _B_in["w2"],
        "gate_w": _w((lambda *s: _rng.normal(s) * 0.05)(1024) * 16.0),
    }

def reference(A_x, A_k_cache, A_v_cache, A_wq, A_wo, B_x, B_w1, B_w2, gate_w):
    def _A_ref(x, k_cache, v_cache, wq, wo):
        B, Sq, D = x.shape
        Hq, Dh = 32, 128
        Hkv, Sk = k_cache.shape[1], k_cache.shape[2]
        W = min(4096, max(256, Sk // 4))
        rep = Hq // Hkv
        q = (lambda x, *d: x.transpose(*d))((x @ wq).reshape(B, Sq, Hq, Dh), 0, 2, 1, 3)
        k = jnp.repeat(k_cache[:, :, Sk - W:, :], rep, axis=1)
        v = jnp.repeat(v_cache[:, :, Sk - W:, :], rep, axis=1)
        scores = jnp.einsum("bhqd,bhkd->bhqk", q, k) * (Dh ** -0.5)
        p = _softmax(scores, axis=-1)
        o = jnp.einsum("bhqk,bhkd->bhqd", p, v)
        return (lambda x, *d: x.transpose(*d))(o, 0, 2, 1, 3).reshape(B, Sq, Hq * Dh) @ wo

    def _B_ref(x, w1, w2):
        h = jnp.einsum("bsd,df->bsf", x, w1)
        h = _silu(h)
        out = jnp.einsum("bsf,fd->bsd", h, w2)
        return out

    x = A_x
    g = _sigmoid((x * gate_w).sum(-1, keepdims=True))
    a = _A_ref(x, A_k_cache, A_v_cache, A_wq, A_wo)
    b = _B_ref(x, B_w1, B_w2)
    return g * a + (1 - g) * b
```

```python
import jax
import jax.numpy as jnp
import jax.experimental.pallas as pl
import jax.experimental.pallas.tpu as pltpu

_LOOK = 4
_HQ, _DH = 32, 128


def _build(B, D, Hkv, Sk, F, look):
    bf, f32 = jnp.bfloat16, jnp.float32
    Hq, Dh = _HQ, _DH
    rep = Hq // Hkv
    W = min(4096, max(256, Sk // 4))
    M = B * rep
    KC, RC = 128, 512
    n_q, n_kv, n_1 = D // KC, B * Hkv, D // KC
    n_o, n_2 = Hq * Dh // RC, F // RC
    hpc = RC // Dh
    scale = Dh ** -0.5
    rnd = lambda t: t.astype(bf).astype(f32)

    def kernel(x_h, k_h, v_h, wq_h, wo_h, w1_h, w2_h, gw_h, out_ref,
               xb, gwb, kb, vb, wqb, wob, w1b, w2b,
               xs, qacc, qs, os_, hacc, hs, aacc, bacc,
               s_x, s_g, s_k, s_v, s_q, s_o, s_1, s_2):
        def rows(src, dst, sem, r):
            def f(i):
                sl = pl.ds(i * r if isinstance(i, int) else pl.multiple_of(i * r, r), r)
                return pltpu.make_async_copy(src.at[sl], dst.at[sl], sem.at[i])
            return f

        def cache(src, dst, sem):
            def f(i):
                b, h = (i // Hkv, i % Hkv)
                return pltpu.make_async_copy(
                    src.at[b, h, pl.ds(Sk - W, W)], dst.at[i], sem.at[i])
            return f

        c_q, c_1 = rows(wq_h, wqb, s_q, KC), rows(w1_h, w1b, s_1, KC)
        c_o, c_2 = rows(wo_h, wob, s_o, RC), rows(w2_h, w2b, s_2, RC)
        c_k, c_v = cache(k_h, kb, s_k), cache(v_h, vb, s_v)
        c_x = pltpu.make_async_copy(x_h, xb, s_x)
        c_g = pltpu.make_async_copy(gw_h, gwb, s_g)

        c_q(0).start()
        c_x.start()
        c_g.start()
        if look:
            for i in range(1, look):
                c_q(i).start()
        else:
            for i in range(1, n_q):
                c_q(i).start()
            for i in range(n_kv):
                c_k(i).start()
                c_v(i).start()
            for c, n in ((c_1, n_1), (c_o, n_o), (c_2, n_2)):
                for i in range(n):
                    c(i).start()

        def ahead(i, step, n, cur, nxt):
            if not look:
                return
            pl.when(i + step < n)(lambda: cur(i + step).start())
            if nxt is not None:
                pl.when(i + step >= n)(lambda: nxt(i + step - n))

        c_x.wait()
        c_g.wait()
        row = jax.lax.broadcasted_iota(jnp.int32, (M, D), 0)
        x16 = jnp.zeros((M, D), f32)
        for b in range(B):
            xrow = xb[b].astype(f32)
            x16 = jnp.where(row // rep == b, xrow, x16)
        for i in range(D // KC):
            xs[i] = x16[:, i * KC:(i + 1) * KC].astype(bf)
        gw = gwb[...].astype(f32).reshape(1, D)
        g = rnd(jax.nn.sigmoid(rnd(jnp.sum(rnd(x16 * gw), axis=-1, keepdims=True))))

        qacc[...] = jnp.zeros_like(qacc)

        def nxt_kv(j):
            pl.when(j % 2 == 0)(lambda: c_k(j // 2).start())
            pl.when(j % 2 == 1)(lambda: c_v(j // 2).start())

        @pl.loop(0, n_q)
        def _(i):
            c_q(i).wait()
            ahead(i, look, n_q, c_q, nxt_kv)
            qacc[...] += jnp.dot(xs[i], wqb[pl.ds(pl.multiple_of(i * KC, KC), KC)],
                                 preferred_element_type=f32)

        r8 = jax.lax.broadcasted_iota(jnp.int32, (M, Dh), 0) % rep
        for h in range(Hkv):
            qh = jnp.zeros((M, Dh), f32)
            for r in range(rep):
                c0 = (h * rep + r) * Dh
                qh = jnp.where(r8 == r, qacc[:, c0:c0 + Dh], qh)
            for b in range(B):
                qs[b * Hkv + h] = qh[b * rep:(b + 1) * rep]

        @pl.loop(0, n_kv)
        def _(i):
            c_k(i).wait()
            ahead(i, look // 2, n_kv, c_k, lambda j: c_1(2 * j).start())
            s = jax.lax.dot_general(qs[i].astype(bf), kb[i], (((1,), (1,)), ((), ())),
                                    preferred_element_type=f32) * scale
            e = jnp.exp(s - jnp.max(s, axis=-1, keepdims=True))
            l = jnp.sum(e, axis=-1, keepdims=True)
            c_v(i).wait()
            ahead(i, look // 2, n_kv, c_v, lambda j: c_1(2 * j + 1).start())
            o = jnp.dot(e.astype(bf), vb[i], preferred_element_type=f32) / l
            os_[i % Hkv, pl.ds(pl.multiple_of((i // Hkv) * rep, rep), rep), :] = o

        hacc[...] = jnp.zeros_like(hacc)

        @pl.loop(0, n_1)
        def _(i):
            c_1(i).wait()
            ahead(i, look, n_1, c_1, lambda j: c_o(j).start())
            hacc[...] += jnp.dot(xs[i], w1b[pl.ds(pl.multiple_of(i * KC, KC), KC)],
                                 preferred_element_type=f32)

        for i in range(n_2):
            hh = rnd(hacc[:, i * RC:(i + 1) * RC])
            hs[i] = (hh * jax.nn.sigmoid(hh)).astype(bf)

        aacc[...] = jnp.zeros_like(aacc)
        rr = jax.lax.broadcasted_iota(jnp.int32, (M, RC), 0) % rep
        cc = jax.lax.broadcasted_iota(jnp.int32, (M, RC), 1) // Dh
        cph = rep // hpc

        @pl.loop(0, n_o)
        def _(i):
            c_o(i).wait()
            ahead(i, look, n_o, c_o, lambda j: c_2(j).start())
            oh = os_[i // cph]
            lhs = jnp.where(rr == cc + (i % cph) * hpc,
                            jnp.concatenate([oh] * hpc, axis=1), 0.0).astype(bf)
            aacc[...] += jnp.dot(lhs, wob[pl.ds(pl.multiple_of(i * RC, RC), RC)],
                                 preferred_element_type=f32)

        bacc[...] = jnp.zeros_like(bacc)

        @pl.loop(0, n_2)
        def _(i):
            c_2(i).wait()
            ahead(i, look, n_2, c_2, None)
            bacc[...] += jnp.dot(hs[i], w2b[pl.ds(pl.multiple_of(i * RC, RC), RC)],
                                 preferred_element_type=f32)

        for b in range(B):
            sl = slice(b * rep, (b + 1) * rep)
            a = rnd(jnp.sum(aacc[sl], axis=0, keepdims=True))
            bb = rnd(bacc[b * rep:b * rep + 1])
            gb = g[b * rep:b * rep + 1]
            out_ref[b] = (rnd(gb * a) + rnd(rnd(1.0 - gb) * bb)).astype(bf)

    vm, dma = pltpu.VMEM, pltpu.SemaphoreType.DMA
    return pl.pallas_call(
        kernel,
        out_shape=jax.ShapeDtypeStruct((B, 1, D), bf),
        in_specs=[pl.BlockSpec(memory_space=pl.ANY)] * 8,
        scratch_shapes=[
            vm((B, 1, D), bf), vm((D,), bf),
            vm((n_kv, W, Dh), bf), vm((n_kv, W, Dh), bf),
            vm((D, Hq * Dh), bf), vm((Hq * Dh, D), bf), vm((D, F), bf), vm((F, D), bf),
            vm((D // KC, M, KC), bf), vm((M, Hq * Dh), f32), vm((n_kv, rep, Dh), f32),
            vm((Hkv, M, Dh), f32), vm((M, F), f32), vm((n_2, M, RC), bf),
            vm((M, D), f32), vm((M, D), f32),
            dma(()), dma(()), dma((n_kv,)), dma((n_kv,)), dma((n_q,)), dma((n_o,)),
            dma((n_1,)), dma((n_2,)),
        ],
        compiler_params=pltpu.CompilerParams(vmem_limit_bytes=64 * 2**20),
    )


@jax.jit
def pallas_gated_mix__sliding_block_cached__dense_activation_silu__decode_kernel(
    A_x: jax.Array,
    A_k_cache: jax.Array,
    A_v_cache: jax.Array,
    A_wq: jax.Array,
    A_wo: jax.Array,
    B_x: jax.Array,
    B_w1: jax.Array,
    B_w2: jax.Array,
    gate_w: jax.Array,
):
    del B_x
    B, _, D = A_x.shape
    _, Hkv, Sk, _ = A_k_cache.shape
    call = _build(B, D, Hkv, Sk, B_w1.shape[1], _LOOK)
    return call(A_x, A_k_cache, A_v_cache, A_wq, A_wo, B_w1, B_w2, gate_w)
```

```python
import jax
import jax.numpy as jnp
import jax.experimental.pallas as pl
import jax.experimental.pallas.tpu as pltpu

_LOOK = 4
_PRIO = True
_TAIL = (384, 128)
_HQ, _DH = 32, 128


def _build(B, D, Hkv, Sk, F, look=_LOOK, prio=_PRIO, tail=_TAIL, KC=128):
    bf, f32 = jnp.bfloat16, jnp.float32
    Hq, Dh = _HQ, _DH
    rep = Hq // Hkv
    W = min(4096, max(256, Sk // 4))
    M = B * rep
    RC = 512
    n_q, n_kv, n_1 = D // KC, B * Hkv, D // KC
    n_o, n_2 = Hq * Dh // RC, F // RC
    hpc = RC // Dh
    scale = Dh ** -0.5
    assert sum(tail) == RC and len(tail) <= look <= n_2 - 1 and B <= 8
    assert all(n % look == 0 for n in (n_q, 2 * n_kv, n_1, n_o))
    rnd = lambda t: t.astype(bf).astype(f32)

    def kernel(x_h, k_h, v_h, wq_h, wo_h, w1_h, w2_h, gw_h, out_ref,
               xb, gwb, kb, vb, wqb, wob, w1b, w2b,
               xs, x8, qacc, qs, os_, hacc, h8, aacc, bacc,
               s_x, s_g, ring):
        def rows(src, dst, r):
            def f(i):
                sl = pl.ds(i * r if isinstance(i, int) else pl.multiple_of(i * r, r), r)
                return pltpu.make_async_copy(src.at[sl], dst.at[sl], ring.at[i % look])
            return f

        def cache(src, dst, off):
            def f(i):
                b, h = (i // Hkv, i % Hkv)
                return pltpu.make_async_copy(
                    src.at[b, h, pl.ds(Sk - W, W)], dst.at[i],
                    ring.at[(2 * i + off) % look])
            return f

        c_q, c_1 = rows(wq_h, wqb, KC), rows(w1_h, w1b, KC)
        c_o, c_2 = rows(wo_h, wob, RC), rows(w2_h, w2b, RC)
        c_k, c_v = cache(k_h, kb, 0), cache(v_h, vb, 1)
        n_2l = n_2 - 1
        t_off = [n_2l * RC + sum(tail[:j]) for j in range(len(tail))]

        def c_t(j):
            sl = pl.ds(t_off[j], tail[j])
            return pltpu.make_async_copy(w2_h.at[sl], w2b.at[sl],
                                         ring.at[(n_2l + j) % look])

        def start(c, j, parity=None):
            if not prio:
                c(j).start()
            elif parity is not None or isinstance(j, int):
                c(j).start(priority=j % 2 if parity is None else parity)
            else:
                pl.when(j % 2 == 0)(lambda: c(j).start(priority=0))
                pl.when(j % 2 == 1)(lambda: c(j).start(priority=1))
        c_x = pltpu.make_async_copy(x_h, xb, s_x)
        c_g = pltpu.make_async_copy(gw_h, gwb, s_g)

        c_q(0).start()
        c_x.start()
        c_g.start()
        for i in range(1, look):
            start(c_q, i)

        def ahead(i, step, n, cur, nxt, parity=None):
            pl.when(i + step < n)(lambda: start(cur, i + step, parity))
            pl.when(i + step >= n)(lambda: nxt(i + step - n))

        c_x.wait()
        c_g.wait()
        row = jax.lax.broadcasted_iota(jnp.int32, (M, D), 0)
        x16 = jnp.zeros((M, D), f32)
        xf = xb[...].astype(f32)
        for b in range(B):
            x16 = jnp.where(row // rep == b, xf[b:b + 1], x16)
        xp = jnp.concatenate([xf, jnp.zeros((8 - B, D), f32)], axis=0)
        for i in range(D // KC):
            x8[i] = xp[:, i * KC:(i + 1) * KC]
            xs[i] = x16[:, i * KC:(i + 1) * KC].astype(bf)
        gw = gwb[...].astype(f32).reshape(1, D)
        g = rnd(jax.nn.sigmoid(rnd(jnp.sum(rnd(x16 * gw), axis=-1, keepdims=True))))

        qacc[...] = jnp.zeros_like(qacc)

        def nxt_kv(j):
            pl.when(j % 2 == 0)(lambda: start(c_k, j // 2, 0))
            pl.when(j % 2 == 1)(lambda: start(c_v, j // 2, 1))

        @pl.loop(0, n_q)
        def _(i):
            c_q(i).wait()
            ahead(i, look, n_q, c_q, nxt_kv)
            qacc[...] += jnp.dot(xs[i], wqb[pl.ds(pl.multiple_of(i * KC, KC), KC)],
                                 preferred_element_type=f32)

        r8 = jax.lax.broadcasted_iota(jnp.int32, (M, Dh), 0) % rep
        for h in range(Hkv):
            qh = jnp.zeros((M, Dh), f32)
            for r in range(rep):
                c0 = (h * rep + r) * Dh
                qh = jnp.where(r8 == r, qacc[:, c0:c0 + Dh], qh)
            for b in range(B):
                qs[b * Hkv + h] = qh[b * rep:(b + 1) * rep]

        @pl.loop(0, n_kv)
        def _(i):
            c_k(i).wait()
            ahead(i, look // 2, n_kv, c_k, lambda j: start(c_1, 2 * j, 0), 0)
            s = jax.lax.dot_general(qs[i].astype(bf), kb[i], (((1,), (1,)), ((), ())),
                                    preferred_element_type=f32) * scale
            e = jnp.exp(s - jnp.max(s, axis=-1, keepdims=True))
            l = jnp.sum(e, axis=-1, keepdims=True)
            c_v(i).wait()
            ahead(i, look // 2, n_kv, c_v, lambda j: start(c_1, 2 * j + 1, 1), 1)
            o = jnp.dot(e.astype(bf), vb[i], preferred_element_type=f32) / l
            os_[i % Hkv, pl.ds(pl.multiple_of((i // Hkv) * rep, rep), rep), :] = o

        hacc[...] = jnp.zeros_like(hacc)

        @pl.loop(0, n_1)
        def _(i):
            c_1(i).wait()
            ahead(i, look, n_1, c_1, lambda j: start(c_o, j))
            hacc[...] += jnp.dot(x8[i].astype(bf), w1b[pl.ds(pl.multiple_of(i * KC, KC), KC)],
                                 preferred_element_type=f32)

        for i in range(n_2):
            hh = rnd(hacc[:, i * RC:(i + 1) * RC])
            h8[i] = hh * jax.nn.sigmoid(hh)

        aacc[...] = jnp.zeros_like(aacc)
        rr = jax.lax.broadcasted_iota(jnp.int32, (M, RC), 0) % rep
        cc = jax.lax.broadcasted_iota(jnp.int32, (M, RC), 1) // Dh
        cph = rep // hpc

        @pl.loop(0, n_o)
        def _(i):
            c_o(i).wait()
            ahead(i, look, n_o, c_o, lambda j: start(c_2, j))
            oh = os_[i // cph]
            lhs = jnp.where(rr == cc + (i % cph) * hpc,
                            jnp.concatenate([oh] * hpc, axis=1), 0.0).astype(bf)
            aacc[...] += jnp.dot(lhs, wob[pl.ds(pl.multiple_of(i * RC, RC), RC)],
                                 preferred_element_type=f32)

        ga, gb = [], []
        for b in range(B):
            gg = g[b * rep:b * rep + 1]
            a = rnd(jnp.sum(aacc[b * rep:(b + 1) * rep], axis=0, keepdims=True))
            ga.append(rnd(gg * a))
            gb.append(rnd(1.0 - gg))
        aacc[0:B] = jnp.concatenate(ga, axis=0)
        gb = jnp.concatenate(gb, axis=0)

        bacc[...] = jnp.zeros_like(bacc)

        def nxt_t(j):
            for t in range(min(look, len(tail))):
                pl.when(j == t)(lambda t=t: c_t(t).start(priority=(n_2l + t) % 2 if prio else 0))

        @pl.loop(0, n_2l)
        def _(i):
            c_2(i).wait()
            ahead(i, look, n_2l, c_2, nxt_t)
            bacc[...] += jnp.dot(h8[i].astype(bf), w2b[pl.ds(pl.multiple_of(i * RC, RC), RC)],
                                 preferred_element_type=f32)

        acc = bacc[...]
        for t in range(len(tail)):
            c_t(t).wait()
            o0 = t_off[t] - n_2l * RC
            acc += jnp.dot(h8[n_2l, :, o0:o0 + tail[t]].astype(bf),
                           w2b[pl.ds(t_off[t], tail[t])],
                           preferred_element_type=f32)
        out_ref[...] = (aacc[0:B] + rnd(gb * rnd(acc[0:B]))).astype(bf)

    vm, dma = pltpu.VMEM, pltpu.SemaphoreType.DMA
    return pl.pallas_call(
        kernel,
        out_shape=jax.ShapeDtypeStruct((B, D), bf),
        in_specs=[pl.BlockSpec(memory_space=pl.ANY)] * 8,
        scratch_shapes=[
            vm((B, D), bf), vm((D,), bf),
            vm((n_kv, W, Dh), bf), vm((n_kv, W, Dh), bf),
            vm((D, Hq * Dh), bf), vm((Hq * Dh, D), bf), vm((D, F), bf), vm((F, D), bf),
            vm((D // KC, M, KC), bf), vm((D // KC, 8, KC), f32),
            vm((M, Hq * Dh), f32), vm((n_kv, rep, Dh), f32),
            vm((Hkv, M, Dh), f32), vm((8, F), f32), vm((n_2, 8, RC), f32),
            vm((M, D), f32), vm((8, D), f32),
            dma(()), dma(()), dma((look,)),
        ],
        compiler_params=pltpu.CompilerParams(vmem_limit_bytes=64 * 2**20),
    )


@jax.jit
def pallas_gated_mix__sliding_block_cached__dense_activation_silu__decode_kernel(
    A_x: jax.Array,
    A_k_cache: jax.Array,
    A_v_cache: jax.Array,
    A_wq: jax.Array,
    A_wo: jax.Array,
    B_x: jax.Array,
    B_w1: jax.Array,
    B_w2: jax.Array,
    gate_w: jax.Array,
):
    del B_x
    B, _, D = A_x.shape
    _, Hkv, Sk, _ = A_k_cache.shape
    call = _build(B, D, Hkv, Sk, B_w1.shape[1])
    out = call(A_x.reshape(B, D), A_k_cache, A_v_cache, A_wq, A_wo, B_w1, B_w2, gate_w)
    return out.reshape(B, 1, D)
```
